```python
import jax
import jax.numpy as jnp

def _softmax(x, axis=-1):
    return jax.nn.softmax(x, axis=axis)
def _gelu(x):
    return jax.nn.gelu(x, approximate=True)
def _silu(x):
    return jax.nn.silu(x)
def _sigmoid(x):
    return jax.nn.sigmoid(x)
def _layernorm(x, axis=-1, eps=1e-5):
    m = jnp.mean(x, axis=axis, keepdims=True)
    v = jnp.var(x, axis=axis, keepdims=True)
    return (x - m) / jnp.sqrt(v + eps)
def _scatter_add(tgt, idx, src, axis=0):
    return tgt.at[idx].add(src)
def _segment_sum(src, seg, n):
    return jax.ops.segment_sum(src, seg, n)
class _Rng:
    def __init__(self, key):
        self._k = key
    def _next(self):
        self._k, sub = jax.random.split(self._k)
        return sub
    def normal(self, shape):
        return jax.random.normal(self._next(), shape, dtype=jnp.bfloat16)
    def randint(self, lo, hi, shape):
        return jax.random.randint(self._next(), shape, lo, hi, dtype=jnp.int32)
    def uniform(self, shape, lo=0.0, hi=1.0):
        return jax.random.uniform(self._next(), shape, jnp.bfloat16, lo, hi)
    def permutation(self, n):
        return jax.random.permutation(self._next(), n)


kernel_name = 'standalone__gqa_block_cached__near_ridge'

def setup_inputs():
    _rng = _Rng(jax.random.key(int.from_bytes(__import__("os").urandom(4), "little")))
    _w = (lambda a: (lambda t: t.astype(jnp.bfloat16) if jnp.issubdtype(t.dtype, jnp.floating) else t)(jnp.asarray(a)))
    B, Sq, D = 16, 240, 640
    Hq, Hkv, Sk, Dh = 32, 32, 1024, 128
    assert Hq % Hkv == 0, (Hq, Hkv)
    return {
        "x": _w((lambda *s: _rng.normal(s) * 0.05)(B, Sq, D)),
        "k_cache": _w((lambda *s: _rng.normal(s) * 0.05)(B, Hkv, Sk, Dh)),
        "v_cache": _w((lambda *s: _rng.normal(s) * 0.05)(B, Hkv, Sk, Dh)),
        "wq": _w((lambda *s: _rng.normal(s) * 0.05)(D, Hq * Dh) * (D ** -0.5)),
        "wo": _w((lambda *s: _rng.normal(s) * 0.05)(Hq * Dh, D) * ((Hq * Dh) ** -0.5)),
    }

def reference(x, k_cache, v_cache, wq, wo):
    B, Sq, D = x.shape
    Hq, Dh = 32, 128
    Hkv = k_cache.shape[1]
    rep = Hq // Hkv
    q = (lambda x, *d: x.transpose(*d))((x @ wq).reshape(B, Sq, Hq, Dh), 0, 2, 1, 3)
    k = jnp.repeat(k_cache, rep, axis=1)
    v = jnp.repeat(v_cache, rep, axis=1)
    scores = jnp.einsum("bhqd,bhkd->bhqk", q, k) * (Dh ** -0.5)
    p = _softmax(scores, axis=-1)
    o = jnp.einsum("bhqk,bhkd->bhqd", p, v)
    return (lambda x, *d: x.transpose(*d))(o, 0, 2, 1, 3).reshape(B, Sq, Hq * Dh) @ wo
```

```python
import math
import jax
import jax.numpy as jnp
from jax import lax
import jax.experimental.pallas as pl
import jax.experimental.pallas.tpu as pltpu

KB = 512


def fine_order(G, ahead=2, pat="1010101010101010", qlead=2, olag=1):
    att = [f"S{u}" for u in range(ahead)]
    U = 2 * G
    for u in range(U):
        if u + ahead < U:
            att.append(f"S{u+ahead}")
        att.append(f"P{u}")
    toks = ["T0", "q0", "q1"]
    qs = []
    for h in range(G):
        if h % 4 == 0:
            qs.append(f"T{h}")
        qs.append(f"q{h}")
    qs = [t for t in qs if t not in toks]
    os_ = []
    for i, tk in enumerate(att):
        u = int(tk[1:])
        if tk[0] == 'S':
            while f"q{u//2}" not in toks:
                toks.append(qs.pop(0))
        toks.append(tk)
        if tk[0] == 'P' and (u + 1) % 8 == 0:
            os_ += [(i + olag, f"o{(u+1)//2-4}-{n}") for n in range(5)]
        if pat[i % 16] == '1':
            urgent = qs and int(qs[0][1:]) <= u // 2 + qlead
            ready = os_ and os_[0][0] <= i
            if urgent or (qs and not ready):
                toks.append(qs.pop(0))
            elif ready:
                toks.append(os_.pop(0)[1])
    toks += [t for _, t in os_]
    return toks


def make(phases=(8, 24), vmem_mb=110, fine={}, NP=4, peel=False):
    def fn(x, k_cache, v_cache, wq, wo):
        B, Sq, D = x.shape
        _, H, Sk, Dh = k_cache.shape
        assert sum(phases) == H
        NPH = len(phases)
        h0s = [sum(phases[:i]) for i in range(NPH)]
        c = (Dh ** -0.5) * math.log2(math.e)
        f32 = jnp.float32

        def kern(x_hbm, k_hbm, v_hbm, wq_hbm, wo_hbm, out_hbm,
                 x_v, wq_v, wo_v, kbuf, vbuf, acc, obuf, p_buf, sx, sw, skv, so):
            def x_cp(b):
                return pltpu.make_async_copy(x_hbm.at[b], x_v.at[b % 2], sx.at[b % 2])

            def wq_cp(h, ph):
                cs = pl.ds(pl.multiple_of(h * Dh, 4 * Dh) if not isinstance(h, int) else h * Dh, 4 * Dh)
                return pltpu.make_async_copy(wq_hbm.at[:, cs], wq_v.at[:, cs], sw.at[ph])

            def wo_cp(h, ph):
                cs = pl.ds(pl.multiple_of(h * Dh, 4 * Dh) if not isinstance(h, int) else h * Dh, 4 * Dh)
                return pltpu.make_async_copy(wo_hbm.at[cs, :], wo_v.at[cs, :], sw.at[ph])

            def kv_cp(ph, b, h=None, n=None):
                hs = pl.ds(h0s[ph], phases[ph]) if h is None else pl.ds(h, n)
                return [pltpu.make_async_copy(src.at[b, hs], dst.at[b % 2, hs], skv.at[2 * ph + b % 2])
                        for src, dst in ((k_hbm, kbuf), (v_hbm, vbuf))]

            def start_in(ph, b):
                x_cp(b).start()
                for cp in kv_cp(ph, b):
                    cp.start()

            def wait_in(ph, b):
                x_cp(b).wait()
                for cp in kv_cp(ph, b):
                    cp.wait()

            def o_cp(b):
                return pltpu.make_async_copy(obuf.at[b % 2], out_hbm.at[b], so.at[b % 2])

            for h in range(0, phases[0], 4):
                wq_cp(h, 0).start()
            start_in(0, 0)
            for h in range(0, phases[0], 4):
                wo_cp(h, 0).start()
            for h in range(0, phases[0], 4):
                wq_cp(h, 0).wait()
                wo_cp(h, 0).wait()
            wait_in(0, 0)
            start_in(0, 1)

            def compute(ph, b):
                G, h0 = phases[ph], h0s[ph]
                slot = b % 2
                tq = {}; q = {}; ms = {}; al = {}; ls = {}; r = {}; o = {}
                for tok in fine_order(G, **fine):
                    kind = tok[0]
                    if kind == 'o':
                        a, e = map(int, tok[1:].split('-'))
                    else:
                        h = int(tok[1:])
                    if kind == 'T':
                        g = h0 + h
                        tt = jnp.dot(x_v[slot, :, 512:], wq_v[512:, g * Dh:(g + 4) * Dh], preferred_element_type=f32)
                        for i in range(4):
                            tq[h + i] = tt[:, i * Dh:(i + 1) * Dh]
                    elif kind == 'q':
                        g = h0 + h
                        qq = jnp.dot(x_v[slot, :, :512], wq_v[:512, g * Dh:(g + 1) * Dh], preferred_element_type=f32)
                        q[h] = ((qq + tq[h]) * c).astype(jnp.bfloat16)
                    elif kind == 'o':
                        oc = jnp.concatenate([o[h] for h in range(a, a + 4)], axis=-1)
                        cs = slice(e * 128, (e + 1) * 128)
                        g = h0 + a
                        yy = jnp.dot(oc, wo_v[g * Dh:(g + 4) * Dh, cs], preferred_element_type=f32)
                        if g > 0:
                            yy = yy + acc[b, :, cs]
                        if g == H - 4:
                            obuf[slot, :, cs] = yy.astype(obuf.dtype)
                        else:
                            acc[b, :, cs] = yy
                    elif kind == 'S':
                        hh, blk = divmod(h, 2)
                        ss = lax.dot_general(q[hh], kbuf[slot, h0 + hh, blk * KB:(blk + 1) * KB], (((1,), (1,)), ((), ())),
                                             preferred_element_type=f32)
                        m = jnp.max(ss, axis=-1, keepdims=True)
                        if blk > 0:
                            m = jnp.maximum(m, ms[hh])
                            al[hh] = jnp.exp2(ms[hh] - m)
                        ms[hh] = m
                        pp = jnp.exp2(ss - m)
                        lp = pp[:, :128]
                        for i in range(1, KB // 128):
                            lp = lp + pp[:, i * 128:(i + 1) * 128]
                        ls[hh] = lp if blk == 0 else al[hh] * ls[hh] + lp
                        if blk == 1:
                            l = jnp.sum(ls[hh], axis=-1, keepdims=True)
                            rr = pl.reciprocal(l, approx=True)
                            r[hh] = rr * (2.0 - l * rr)
                        p_buf[h % NP] = pp.astype(jnp.bfloat16)
                    elif kind == 'P':
                        hh, blk = divmod(h, 2)
                        oo = jnp.dot(p_buf[h % NP], vbuf[slot, h0 + hh, blk * KB:(blk + 1) * KB], preferred_element_type=f32)
                        if blk == 0:
                            o[hh] = oo
                        else:
                            o[hh] = ((al[hh] * o[hh] + oo) * r[hh]).astype(jnp.bfloat16)

            for ph in range(NPH):
                last = ph == NPH - 1

                def body(b, carry, ph=ph, last=last):
                    compute(ph, b)

                    @pl.when(b + 1 < B)
                    def _():
                        wait_in(ph, b + 1)

                    @pl.when(b + 2 < B)
                    def _():
                        start_in(ph, b + 2)

                    if not last:
                        Gn, hn = phases[ph + 1], h0s[ph + 1]
                        n4 = Gn // 4

                        @pl.when(b < n4)
                        def _():
                            wq_cp(hn + 4 * b, ph + 1).start()

                        @pl.when(jnp.logical_and(b >= n4, b < 2 * n4))
                        def _():
                            wo_cp(hn + 4 * (b - n4), ph + 1).start()

                        @pl.when(b < Gn // 2)
                        def _():
                            for cp in kv_cp(ph + 1, 0, hn + 2 * b, 2):
                                cp.start()

                        @pl.when(b == B - 2)
                        def _():
                            x_cp(0).start()

                        @pl.when(b == B - 1)
                        def _():
                            for h in range(hn, hn + Gn, 4):
                                wq_cp(h, ph + 1).wait()
                                wo_cp(h, ph + 1).wait()
                            wait_in(ph + 1, 0)
                            start_in(ph + 1, 1)
                    else:
                        o_cp(b).start()

                        @pl.when(b >= 1)
                        def _():
                            o_cp(b - 1).wait()
                    return carry

                lax.fori_loop(0, B, body, 0)
            o_cp(B - 1).wait()

        any_spec = pl.BlockSpec(memory_space=pl.ANY)
        return pl.pallas_call(
            kern,
            in_specs=[any_spec] * 5,
            out_specs=any_spec,
            out_shape=jax.ShapeDtypeStruct((B, Sq, D), x.dtype),
            scratch_shapes=[
                pltpu.VMEM((2, Sq, D), x.dtype),
                pltpu.VMEM(wq.shape, wq.dtype),
                pltpu.VMEM(wo.shape, wo.dtype),
                pltpu.VMEM((2, H, Sk, Dh), k_cache.dtype),
                pltpu.VMEM((2, H, Sk, Dh), v_cache.dtype),
                pltpu.VMEM((B, Sq, D), f32),
                pltpu.VMEM((2, Sq, D), x.dtype),
                pltpu.VMEM((NP, Sq, KB), jnp.bfloat16),
                pltpu.SemaphoreType.DMA((2,)),
                pltpu.SemaphoreType.DMA((NPH,)),
                pltpu.SemaphoreType.DMA((2 * NPH,)),
                pltpu.SemaphoreType.DMA((2,)),
            ],
            compiler_params=pltpu.CompilerParams(
                vmem_limit_bytes=vmem_mb * 1024 * 1024,
                disable_bounds_checks=True,
            ),
        )(x, k_cache, v_cache, wq, wo)
    return fn


@jax.jit
def pallas_standalone__gqa_block_cached__near_ridge_kernel(x, k_cache, v_cache, wq, wo):
    return make()(x, k_cache, v_cache, wq, wo)
```

```python
import math
import jax
import jax.numpy as jnp
from jax import lax
import jax.experimental.pallas as pl
import jax.experimental.pallas.tpu as pltpu

KB = 512


def fine_order(G, ahead=2, pat="1010101010101010", qlead=2, olag=1):
    att = [f"S{u}" for u in range(ahead)]
    U = 2 * G
    for u in range(U):
        if u + ahead < U:
            att.append(f"S{u+ahead}")
        att.append(f"P{u}")
    toks = ["T0", "q0", "q1"]
    qs = []
    for h in range(G):
        if h % 4 == 0:
            qs.append(f"T{h}")
        qs.append(f"q{h}")
    qs = [t for t in qs if t not in toks]
    os_ = []
    for i, tk in enumerate(att):
        u = int(tk[1:])
        if tk[0] == 'S':
            while f"q{u//2}" not in toks:
                toks.append(qs.pop(0))
        toks.append(tk)
        if tk[0] == 'P' and (u + 1) % 8 == 0:
            os_ += [(i + olag, f"o{(u+1)//2-4}-{n}") for n in range(5)]
        if pat[i % 16] == '1':
            urgent = qs and int(qs[0][1:]) <= u // 2 + qlead
            ready = os_ and os_[0][0] <= i
            if urgent or (qs and not ready):
                toks.append(qs.pop(0))
            elif ready:
                toks.append(os_.pop(0)[1])
    toks += [t for _, t in os_]
    return toks


def make(phases=(8, 24), vmem_mb=110, fine={}, NP=4, peel=(((0, 2), (0,), ()), ((2, 4), (1,), ()), ((4, 8), (), (0, 1))), pre=2, PW=512, flags=None):
    def fn(x, k_cache, v_cache, wq, wo):
        B, Sq, D = x.shape
        _, H, Sk, Dh = k_cache.shape
        assert sum(phases) == H
        NPH = len(phases)
        h0s = [sum(phases[:i]) for i in range(NPH)]
        c = (Dh ** -0.5) * math.log2(math.e)
        f32 = jnp.float32

        def kern(x_hbm, k_hbm, v_hbm, wq_hbm, wo_hbm, out_hbm,
                 x_v, wq_v, wo_v, kbuf, vbuf, acc, obuf, p_buf, sx, sw, skv, so, sp):
            def x_cp(b):
                return pltpu.make_async_copy(x_hbm.at[b], x_v.at[b % 2], sx.at[b % 2])

            def wq_cp(h, ph):
                cs = pl.ds(pl.multiple_of(h * Dh, 4 * Dh) if not isinstance(h, int) else h * Dh, 4 * Dh)
                return pltpu.make_async_copy(wq_hbm.at[:, cs], wq_v.at[:, cs], sw.at[ph])

            def wo_cp(h, ph):
                cs = pl.ds(pl.multiple_of(h * Dh, 4 * Dh) if not isinstance(h, int) else h * Dh, 4 * Dh)
                return pltpu.make_async_copy(wo_hbm.at[cs, :], wo_v.at[cs, :], sw.at[ph])

            def kv_cp(ph, b, h=None, n=None):
                hs = pl.ds(h0s[ph], phases[ph]) if h is None else pl.ds(h, n)
                return [pltpu.make_async_copy(src.at[b, hs], dst.at[b % 2, hs], skv.at[2 * ph + b % 2])
                        for src, dst in ((k_hbm, kbuf), (v_hbm, vbuf))]

            def start_in(ph, b):
                x_cp(b).start()
                for cp in kv_cp(ph, b):
                    cp.start()

            def wait_in(ph, b):
                x_cp(b).wait()
                for cp in kv_cp(ph, b):
                    cp.wait()

            def o_cp(b):
                return pltpu.make_async_copy(obuf.at[b % 2], out_hbm.at[b], so.at[b % 2])

            if not peel:
                for h in range(0, phases[0], 4):
                    wq_cp(h, 0).start()
                start_in(0, 0)
                for h in range(0, phases[0], 4):
                    wo_cp(h, 0).start()
                for h in range(0, phases[0], 4):
                    wq_cp(h, 0).wait()
                    wo_cp(h, 0).wait()
                wait_in(0, 0)
                start_in(0, 1)
            else:
                def stage(i):
                    hs, qg, og = peel[i]
                    cps = [x_cp(0)] if i == 0 else []
                    for g in qg:
                        cs = pl.ds(g * 4 * Dh, 4 * Dh)
                        cps.append(pltpu.make_async_copy(wq_hbm.at[:, cs], wq_v.at[:, cs], sp.at[i]))
                    hsl = pl.ds(hs[0], hs[1] - hs[0])
                    cps += [pltpu.make_async_copy(src.at[0, hsl], dst.at[0, hsl], sp.at[i])
                            for src, dst in ((k_hbm, kbuf), (v_hbm, vbuf))]
                    for g in og:
                        cs = pl.ds(g * 4 * Dh, 4 * Dh)
                        cps.append(pltpu.make_async_copy(wo_hbm.at[cs, :], wo_v.at[cs, :], sp.at[i]))
                    return cps

                def stage_of(tok):
                    kind = tok[0]
                    n = int(tok[1:].split('-')[0])
                    for i, (hs, qg, og) in enumerate(peel):
                        if kind in 'SP' and hs[0] <= n // 2 < hs[1]:
                            return i
                        if kind in 'Tq' and n // 4 in qg:
                            return i
                        if kind == 'o' and n // 4 in og:
                            return i

                for i in range(min(len(peel), pre)):
                    for cp in stage(i):
                        cp.start()
                if pre > len(peel):
                    start_in(0, 1)

            def compute(ph, b, first=False):
                ready = -1
                G, h0 = phases[ph], h0s[ph]
                slot = b % 2
                tq = {}; q = {}; ms = {}; al = {}; ls = {}; r = {}; o = {}
                for tok in fine_order(G, **fine):
                    kind = tok[0]
                    while first and ready < stage_of(tok):
                        ready += 1
                        for cp in stage(ready):
                            cp.wait()
                        if ready + pre < len(peel):
                            for cp in stage(ready + pre):
                                cp.start()
                        elif ready + pre == len(peel):
                            start_in(0, 1)
                    if kind == 'o':
                        a, e = map(int, tok[1:].split('-'))
                    else:
                        h = int(tok[1:])
                    if kind == 'T':
                        g = h0 + h
                        tt = jnp.dot(x_v[slot, :, 512:], wq_v[512:, g * Dh:(g + 4) * Dh], preferred_element_type=f32)
                        for i in range(4):
                            tq[h + i] = tt[:, i * Dh:(i + 1) * Dh]
                    elif kind == 'q':
                        g = h0 + h
                        qq = jnp.dot(x_v[slot, :, :512], wq_v[:512, g * Dh:(g + 1) * Dh], preferred_element_type=f32)
                        q[h] = ((qq + tq[h]) * c).astype(jnp.bfloat16)
                    elif kind == 'o':
                        oc = jnp.concatenate([o[h] for h in range(a, a + 4)], axis=-1)
                        cs = slice(e * 128, (e + 1) * 128)
                        g = h0 + a
                        yy = jnp.dot(oc, wo_v[g * Dh:(g + 4) * Dh, cs], preferred_element_type=f32)
                        if g > 0:
                            yy = yy + acc[b, :, cs]
                        if g == H - 4:
                            obuf[slot, :, cs] = yy.astype(obuf.dtype)
                        else:
                            acc[b, :, cs] = yy
                    elif kind == 'S':
                        hh, blk = divmod(h, 2)
                        ss = lax.dot_general(q[hh], kbuf[slot, h0 + hh, blk * KB:(blk + 1) * KB], (((1,), (1,)), ((), ())),
                                             preferred_element_type=f32)
                        m = jnp.max(ss, axis=-1, keepdims=True)
                        if blk > 0:
                            m = jnp.maximum(m, ms[hh])
                            al[hh] = jnp.exp2(ms[hh] - m)
                        ms[hh] = m
                        pp = jnp.exp2(ss - m)
                        lp = pp[:, :128]
                        for i in range(1, KB // 128):
                            lp = lp + pp[:, i * 128:(i + 1) * 128]
                        ls[hh] = lp if blk == 0 else al[hh] * ls[hh] + lp
                        if blk == 1:
                            l = jnp.sum(ls[hh], axis=-1, keepdims=True)
                            rr = pl.reciprocal(l, approx=True)
                            r[hh] = rr * (2.0 - l * rr)
                        pb = pp.astype(jnp.bfloat16)
                        for i in range(KB // PW):
                            p_buf[h % NP, i] = pb[:, i * PW:(i + 1) * PW]
                    elif kind == 'P':
                        hh, blk = divmod(h, 2)
                        oo = jnp.dot(jnp.concatenate([p_buf[h % NP, i] for i in range(KB // PW)], -1), vbuf[slot, h0 + hh, blk * KB:(blk + 1) * KB], preferred_element_type=f32)
                        if blk == 0:
                            o[hh] = oo
                        else:
                            o[hh] = ((al[hh] * o[hh] + oo) * r[hh]).astype(jnp.bfloat16)

            for ph in range(NPH):
                last = ph == NPH - 1

                def body(b, carry, ph=ph, last=last, first=False):
                    compute(ph, b, first)

                    @pl.when(b + 1 < B)
                    def _():
                        wait_in(ph, b + 1)

                    @pl.when(b + 2 < B)
                    def _():
                        start_in(ph, b + 2)

                    if not last:
                        Gn, hn = phases[ph + 1], h0s[ph + 1]
                        n4 = Gn // 4

                        @pl.when(b < n4)
                        def _():
                            wq_cp(hn + 4 * b, ph + 1).start()

                        @pl.when(jnp.logical_and(b >= n4, b < 2 * n4))
                        def _():
                            wo_cp(hn + 4 * (b - n4), ph + 1).start()

                        @pl.when(b < Gn // 2)
                        def _():
                            for cp in kv_cp(ph + 1, 0, hn + 2 * b, 2):
                                cp.start()

                        @pl.when(b == B - 2)
                        def _():
                            x_cp(0).start()

                        @pl.when(b == B - 1)
                        def _():
                            for h in range(hn, hn + Gn, 4):
                                wq_cp(h, ph + 1).wait()
                                wo_cp(h, ph + 1).wait()
                            x_cp(0).wait()
                            for h in range(hn, hn + Gn, 2):
                                for cp in kv_cp(ph + 1, 0, h, 2):
                                    cp.wait()
                            start_in(ph + 1, 1)
                    else:
                        o_cp(b).start()

                        @pl.when(b >= 1)
                        def _():
                            o_cp(b - 1).wait()
                    return carry

                if peel and ph == 0:
                    body(0, 0, first=True)
                    lax.fori_loop(1, B, body, 0)
                else:
                    lax.fori_loop(0, B, body, 0)
            o_cp(B - 1).wait()

        any_spec = pl.BlockSpec(memory_space=pl.ANY)
        return pl.pallas_call(
            kern,
            in_specs=[any_spec] * 5,
            out_specs=any_spec,
            out_shape=jax.ShapeDtypeStruct((B, Sq, D), x.dtype),
            scratch_shapes=[
                pltpu.VMEM((2, Sq, D), x.dtype),
                pltpu.VMEM(wq.shape, wq.dtype),
                pltpu.VMEM(wo.shape, wo.dtype),
                pltpu.VMEM((2, H, Sk, Dh), k_cache.dtype),
                pltpu.VMEM((2, H, Sk, Dh), v_cache.dtype),
                pltpu.VMEM((B, Sq, D), f32),
                pltpu.VMEM((2, Sq, D), x.dtype),
                pltpu.VMEM((NP, KB // PW, Sq, PW), jnp.bfloat16),
                pltpu.SemaphoreType.DMA((2,)),
                pltpu.SemaphoreType.DMA((NPH,)),
                pltpu.SemaphoreType.DMA((2 * NPH,)),
                pltpu.SemaphoreType.DMA((2,)),
                pltpu.SemaphoreType.DMA((8,)),
            ],
            compiler_params=pltpu.CompilerParams(
                vmem_limit_bytes=vmem_mb * 1024 * 1024,
                disable_bounds_checks=True, flags=flags,
            ),
        )(x, k_cache, v_cache, wq, wo)
    return fn


@jax.jit
def pallas_standalone__gqa_block_cached__near_ridge_kernel(x, k_cache, v_cache, wq, wo):
    return make()(x, k_cache, v_cache, wq, wo)
```
